```python
import os as _os
_os.environ.setdefault("JAX_PLATFORMS", "cpu")
import jax
import jax.numpy as jnp

def _softmax(x, axis=-1):
    return jax.nn.softmax(x, axis=axis)
def _gelu(x):
    return jax.nn.gelu(x, approximate=True)
def _silu(x):
    return jax.nn.silu(x)
def _sigmoid(x):
    return jax.nn.sigmoid(x)
def _layernorm(x, axis=-1, eps=1e-5):
    m = jnp.mean(x, axis=axis, keepdims=True)
    v = jnp.var(x, axis=axis, keepdims=True)
    return (x - m) / jnp.sqrt(v + eps)
def _scatter_add(tgt, idx, src, axis=0):
    return tgt.at[idx].add(src)
def _segment_sum(src, seg, n):
    return jax.ops.segment_sum(src, seg, n)
class _Rng:
    def __init__(self, key):
        self._k = key
    def _next(self):
        self._k, sub = jax.random.split(self._k)
        return sub
    def normal(self, shape):
        return jax.random.normal(self._next(), shape, dtype=jnp.bfloat16)
    def randint(self, lo, hi, shape):
        return jax.random.randint(self._next(), shape, lo, hi, dtype=jnp.int32)
    def uniform(self, shape, lo=0.0, hi=1.0):
        return jax.random.uniform(self._next(), shape, jnp.bfloat16, lo, hi)
    def permutation(self, n):
        return jax.random.permutation(self._next(), n)


kernel_name = 'standalone__mha_softmax__decode'

def setup_inputs():
    _rng = _Rng(jax.random.key(int.from_bytes(__import__("os").urandom(4), "little")))
    _w = (lambda a: (lambda t: t.astype(jnp.bfloat16) if jnp.issubdtype(t.dtype, jnp.floating) else t)(jnp.asarray(a)))
    B, H, Sq, Sk, D = 1, 32, 1, 8192, 128
    return {
        "q": _w((lambda *s: _rng.normal(s) * 0.8)(B, H, Sq, D)),
        "k": _w((lambda *s: _rng.normal(s) * 0.8)(B, H, Sk, D)),
        "v": _w((lambda *s: _rng.normal(s) * 0.05)(B, H, Sk, D)),
    }

def reference(q, k, v):
    scale = q.shape[-1] ** -0.5
    scores = jnp.einsum("bhqd,bhkd->bhqk", q, k) * scale
    p = _softmax(scores, axis=-1)
    return jnp.einsum("bhqk,bhkd->bhqd", p, v)
```

```python
import jax
import jax.numpy as jnp
from jax import lax
import jax.experimental.pallas as pl
import jax.experimental.pallas.tpu as pltpu

_HEADS_PER_BLOCK = 16
_DMA_ROWS = 64
_GROUP_KEYS = 128
_RING = 4
_PRIORITY = (0, 1, 1, 1)

_NT = (((1,), (1,)), ((), ()))
_NN = (((1,), (0,)), ((), ()))


@jax.jit
def pallas_standalone__mha_softmax__decode_kernel(
    q: jax.Array,
    k: jax.Array,
    v: jax.Array,
):
    b, h, sq, d = q.shape
    sk = k.shape[2]
    assert sq == 1 and d == 128
    nh = b * h
    hb, cr, gk, nb = _HEADS_PER_BLOCK, _DMA_ROWS, _GROUP_KEYS, _RING
    assert nh % hb == 0 and sk % gk == 0
    ng = sk // gk
    nsub = hb // 8
    look = nb - 1
    scale = d**-0.5
    phases = [(w, blk) for blk in range(nh // hb) for w in range(2)]

    def kernel(q_hbm, k_hbm, v_hbm, o_ref, q_buf, buf, scores, sems, q_sem):
        def start(w, blk, g, slot):
            src = (k_hbm, v_hbm)[w]
            i = 0
            for t in range(gk // cr):
                for s in range(hb):
                    pltpu.make_async_copy(
                        src.at[blk * hb + s, pl.ds(pl.multiple_of(g * gk + t * cr, cr), cr)],
                        buf.at[slot, s, pl.ds(t * cr, cr)],
                        sems.at[slot],
                    ).start(priority=_PRIORITY[i % len(_PRIORITY)])
                    i += 1

        q_copy = pltpu.make_async_copy(q_hbm, q_buf, q_sem)
        start(0, 0, 0, 0)
        q_copy.start()
        lax.fori_loop(1, look, lambda g, _: start(0, 0, g, g), None)
        q_copy.wait()
        row = lax.broadcasted_iota(jnp.int32, (8, d), 0)

        def step(w, blk, g, gi, nxt, carry):
            slot = gi % nb
            pltpu.make_async_copy(buf.at[slot], buf.at[slot], sems.at[slot]).wait()
            if nxt is not None:
                start(*nxt, (gi + look) % nb)
            new = []
            for j in range(nsub):
                if w == 0:
                    lhs = q_buf[pl.ds(blk * hb, hb), :].astype(jnp.float32)
                    lhs = lhs[8 * j : 8 * j + 8].astype(q_buf.dtype)
                else:
                    m, l, acc = carry[j]
                    p = jnp.exp(scores[blk * nsub + j, g] - m)
                    lhs = p.astype(buf.dtype)
                res = None
                for s in range(8):
                    r = lax.dot_general(
                        lhs, buf[slot, 8 * j + s], _NT if w == 0 else _NN,
                        preferred_element_type=jnp.float32,
                    )
                    res = r if res is None else jnp.where(row == s, r, res)
                if w == 0:
                    res = res * scale
                    scores[blk * nsub + j, g] = res
                    new.append(jnp.maximum(carry[j], res))
                else:
                    new.append((m, l + p, acc + res))
            return tuple(new)

        row_max = None
        for pi, (w, blk) in enumerate(phases):
            if w == 0:
                carry = tuple(jnp.full((8, gk), -jnp.inf, jnp.float32) for _ in range(nsub))
            else:
                carry = tuple(
                    (row_max[j], jnp.zeros((8, gk), jnp.float32), jnp.zeros((8, d), jnp.float32))
                    for j in range(nsub)
                )
            carry = lax.fori_loop(
                0, ng - look, lambda g, c: step(w, blk, g, pi * ng + g, (w, blk, g + look), c), carry
            )
            if pi + 1 < len(phases):
                w2, blk2 = phases[pi + 1]
                carry = lax.fori_loop(
                    ng - look, ng,
                    lambda g, c: step(w, blk, g, pi * ng + g, (w2, blk2, g + look - ng), c), carry,
                )
            else:
                carry = lax.fori_loop(
                    ng - look, ng, lambda g, c: step(w, blk, g, pi * ng + g, None, c), carry
                )
            if w == 0:
                row_max = [
                    jnp.broadcast_to(jnp.max(m, axis=1, keepdims=True), (8, gk)) for m in carry
                ]
            else:
                o = [acc / jnp.sum(l, axis=1, keepdims=True) for (_, l, acc) in carry]
                o_ref[pl.ds(blk * hb, hb), :] = jnp.concatenate(o, axis=0).astype(o_ref.dtype)

    out = pl.pallas_call(
        kernel,
        in_specs=[pl.BlockSpec(memory_space=pl.ANY)] * 3,
        out_specs=pl.BlockSpec(memory_space=pltpu.VMEM),
        out_shape=jax.ShapeDtypeStruct((nh, d), q.dtype),
        scratch_shapes=[
            pltpu.VMEM((nh, d), q.dtype),
            pltpu.VMEM((nb, hb, gk, d), k.dtype),
            pltpu.VMEM((nh // 8, ng, 8, gk), jnp.float32),
            pltpu.SemaphoreType.DMA((nb,)),
            pltpu.SemaphoreType.DMA(()),
        ],
        compiler_params=pltpu.CompilerParams(disable_bounds_checks=True),
    )(q.reshape(nh, d), k.reshape(nh, sk, d), v.reshape(nh, sk, d))
    return out.reshape(b, h, sq, d)
```

```python
import jax
import jax.numpy as jnp
from jax import lax
import jax.experimental.pallas as pl
import jax.experimental.pallas.tpu as pltpu

_HEADS = 8
_ROWS = 64
_STREAMS = 2 * _HEADS
_ROUNDS = 2
_PIECES = _ROUNDS * _STREAMS
_SLOTS = 8
_AHEAD = 4
_SEGMENTS = ((0, 16), (16, 26), (26, 32))

_QK = (((1,), (1,)), ((), ()))
_PV = (((1,), (0,)), ((), ()))


def _attention_kernel(
    q_hbm, k_hbm, v_hbm, o_hbm,
    ring, scores, q_f32, row_max, denom, numer, p_cols, o_vmem,
    ring_sems, q_sem, o_sem,
    *, scale,
):
    n_blocks = q_f32.shape[0]
    n_groups = scores.shape[0]
    n_rounds = k_hbm.shape[1] // _ROWS
    groups_per_block = n_rounds // _ROUNDS
    sublane = lax.broadcasted_iota(jnp.int32, (_HEADS, 2 * _ROWS), 0)

    def block_of(g):
        return g >> (groups_per_block.bit_length() - 1)

    def slot_of(g):
        return g & (_SLOTS - 1)

    def enqueue(main, side):
        for piece in range(_PIECES):
            on_main = piece % 4 != 1
            what = main if on_main else side
            if what is None:
                continue
            src, g = what
            rnd = _ROUNDS * (g & (groups_per_block - 1)) + piece // _STREAMS
            first_key = pl.multiple_of((n_rounds - 1 - rnd) * _ROWS, _ROWS)
            seg = next(i for i, (_, hi) in enumerate(_SEGMENTS) if piece < hi)
            pltpu.make_async_copy(
                src.at[block_of(g) * _STREAMS + piece % _STREAMS, pl.ds(first_key, _ROWS)],
                ring.at[slot_of(g), pl.ds(piece * _ROWS, _ROWS)],
                ring_sems.at[slot_of(g) * len(_SEGMENTS) + seg],
            ).start(priority=int(on_main))

    def wait_segment(g, seg):
        lo, hi = _SEGMENTS[seg]
        filled = ring.at[slot_of(g), pl.ds(lo * _ROWS, (hi - lo) * _ROWS)]
        pltpu.make_async_copy(
            filled, filled, ring_sems.at[slot_of(g) * len(_SEGMENTS) + seg]
        ).wait()

    def matmul_round(lhs, g, rnd, dims):
        out = None
        for h in range(_HEADS):
            tile = ring[slot_of(g), pl.ds((rnd * _HEADS + h) * 2 * _ROWS, 2 * _ROWS)]
            res = lax.dot_general(lhs, tile, dims, preferred_element_type=jnp.float32)
            out = res if out is None else jnp.where(sublane == h, res, out)
        return out

    q_land = ring.at[_SLOTS - 1, pl.ds(0, q_hbm.shape[0])]
    q_copy = pltpu.make_async_copy(q_hbm, q_land, q_sem)
    enqueue((k_hbm, 0), None)
    q_copy.start()
    lax.fori_loop(1, _AHEAD, lambda i, _: enqueue((k_hbm, i), (k_hbm, i - 1)), None)
    q_copy.wait()
    q_all = q_land[...].astype(jnp.float32)
    for b in range(n_blocks):
        q_f32[b] = q_all[b * _HEADS : (b + 1) * _HEADS]
    row_max[...] = jnp.full(row_max.shape, -jnp.inf, jnp.float32)
    denom[...] = jnp.zeros(denom.shape, jnp.float32)
    numer[...] = jnp.zeros(numer.shape, jnp.float32)

    def score_step(g, _):
        for seg in range(len(_SEGMENTS)):
            wait_segment(g, seg)
        i = g + _AHEAD
        pl.when(i < n_groups)(lambda: enqueue((k_hbm, i), (k_hbm, i - 1)))
        pl.when(i == n_groups)(lambda: enqueue((v_hbm, 0), (k_hbm, n_groups - 1)))
        pl.when(i > n_groups)(
            lambda: enqueue((v_hbm, i - n_groups), (v_hbm, i - n_groups - 1))
        )
        b = block_of(g)
        q_blk = q_f32[b].astype(ring.dtype)
        m = row_max[b]
        for rnd in range(_ROUNDS):
            s = matmul_round(q_blk, g, rnd, _QK) * scale
            scores[g, rnd] = s
            m = jnp.maximum(m, s)
        row_max[b] = m

    lax.fori_loop(0, n_groups, score_step, None)
    for b in range(n_blocks):
        row_max[b] = jnp.broadcast_to(
            jnp.max(row_max[b], axis=1, keepdims=True), row_max.shape[1:]
        )

    last = n_groups - 1
    p_last = [jnp.exp(scores[last, rnd] - row_max[n_blocks - 1]) for rnd in range(_ROUNDS)]
    denom[n_blocks - 1] = p_last[0] + p_last[1]
    p_last_t = p_last[1].T
    for h in range(_HEADS):
        p_cols[pl.ds(h * 2 * _ROWS, 2 * _ROWS)] = jnp.broadcast_to(
            p_last_t[:, h : h + 1], (2 * _ROWS, p_cols.shape[1])
        )

    def value_step(g, _):
        for seg in range(len(_SEGMENTS)):
            wait_segment(g, seg)
        i = g + _AHEAD
        pl.when(i < n_groups)(lambda: enqueue((v_hbm, i), (v_hbm, i - 1)))
        pl.when(i == n_groups)(lambda: enqueue(None, (v_hbm, n_groups - 1)))
        b = block_of(g)
        m, l, acc = row_max[b], denom[b], numer[b]
        for rnd in range(_ROUNDS):
            p = jnp.exp(scores[g, rnd] - m)
            l = l + p
            acc = acc + matmul_round(p.astype(ring.dtype), g, rnd, _PV)
        denom[b] = l
        numer[b] = acc

    lax.fori_loop(0, last, value_step, None)

    inv = [1.0 / jnp.sum(denom[b], axis=1, keepdims=True) for b in range(n_blocks)]
    done = [numer[b] * inv[b] for b in range(n_blocks - 1)]
    n_early = (n_blocks - 2) * _HEADS
    o_vmem[pl.ds(0, n_early)] = jnp.concatenate(done[:-1], axis=0).astype(o_vmem.dtype)

    wait_segment(last, 0)
    acc = numer[n_blocks - 1] + matmul_round(p_last[0].astype(ring.dtype), last, 0, _PV)
    for seg in range(1, len(_SEGMENTS)):
        wait_segment(last, seg)
        lo, hi = _SEGMENTS[seg]
        for h in range((lo - _STREAMS) // 2, (hi - _STREAMS) // 2):
            tile = ring[slot_of(last), pl.ds((_HEADS + h) * 2 * _ROWS, 2 * _ROWS)]
            prod = p_cols[pl.ds(h * 2 * _ROWS, 2 * _ROWS)] * tile.astype(jnp.float32)
            parts = [prod[j : j + 8] for j in range(0, 2 * _ROWS, 8)]
            while len(parts) > 1:
                parts = [a + b for a, b in zip(parts[0::2], parts[1::2])]
            head_sum = jnp.sum(parts[0], axis=0, keepdims=True)
            acc = jnp.where(sublane == h, acc + head_sum, acc)
    o_vmem[pl.ds(n_early, 2 * _HEADS)] = jnp.concatenate(
        [done[-1], acc * inv[-1]], axis=0
    ).astype(o_vmem.dtype)

    o_copy = pltpu.make_async_copy(o_vmem, o_hbm, o_sem)
    o_copy.start()
    o_copy.wait()


@jax.jit
def pallas_standalone__mha_softmax__decode_kernel(
    q: jax.Array,
    k: jax.Array,
    v: jax.Array,
):
    b, h, sq, d = q.shape
    sk = k.shape[2]
    heads = b * h
    n_blocks = heads // _HEADS
    groups_per_block = sk // (2 * _ROWS * _ROUNDS)
    n_groups = n_blocks * groups_per_block
    assert sq == 1 and d == 2 * _ROWS
    assert heads % (2 * _HEADS) == 0 and n_blocks > 2
    assert sk == groups_per_block * 2 * _ROWS * _ROUNDS
    assert groups_per_block & (groups_per_block - 1) == 0 and n_groups % _SLOTS == 0

    per_block = pltpu.VMEM((n_blocks, _HEADS, d), jnp.float32)
    out = pl.pallas_call(
        lambda *refs: _attention_kernel(*refs, scale=d**-0.5),
        in_specs=[pl.BlockSpec(memory_space=pl.ANY)] * 3,
        out_specs=pl.BlockSpec(memory_space=pl.ANY),
        out_shape=jax.ShapeDtypeStruct((heads, d), q.dtype),
        scratch_shapes=[
            pltpu.VMEM((_SLOTS, _PIECES * _ROWS, d), k.dtype),
            pltpu.VMEM((n_groups, _ROUNDS, _HEADS, 2 * _ROWS), jnp.float32),
            per_block,
            per_block,
            per_block,
            per_block,
            pltpu.VMEM((_STREAMS * _ROWS, d), jnp.float32),
            pltpu.VMEM((heads, d), q.dtype),
            pltpu.SemaphoreType.DMA((_SLOTS * len(_SEGMENTS),)),
            pltpu.SemaphoreType.DMA(()),
            pltpu.SemaphoreType.DMA(()),
        ],
        compiler_params=pltpu.CompilerParams(
            disable_bounds_checks=True, disable_semaphore_checks=True
        ),
        name="mha_softmax_decode",
    )(
        q.reshape(heads, d),
        k.reshape(2 * heads, sk // 2, d),
        v.reshape(2 * heads, sk // 2, d),
    )
    return out.reshape(b, h, sq, d)
```
